```python
import os as _os
_os.environ.setdefault("JAX_PLATFORMS", "cpu")
import jax
import jax.numpy as jnp

def _softmax(x, axis=-1):
    return jax.nn.softmax(x, axis=axis)
def _gelu(x):
    return jax.nn.gelu(x, approximate=True)
def _silu(x):
    return jax.nn.silu(x)
def _sigmoid(x):
    return jax.nn.sigmoid(x)
def _layernorm(x, axis=-1, eps=1e-5):
    m = jnp.mean(x, axis=axis, keepdims=True)
    v = jnp.var(x, axis=axis, keepdims=True)
    return (x - m) / jnp.sqrt(v + eps)
def _scatter_add(tgt, idx, src, axis=0):
    return tgt.at[idx].add(src)
def _segment_sum(src, seg, n):
    return jax.ops.segment_sum(src, seg, n)
class _Rng:
    def __init__(self, key):
        self._k = key
    def _next(self):
        self._k, sub = jax.random.split(self._k)
        return sub
    def normal(self, shape):
        return jax.random.normal(self._next(), shape, dtype=jnp.bfloat16)
    def randint(self, lo, hi, shape):
        return jax.random.randint(self._next(), shape, lo, hi, dtype=jnp.int32)
    def uniform(self, shape, lo=0.0, hi=1.0):
        return jax.random.uniform(self._next(), shape, jnp.bfloat16, lo, hi)
    def permutation(self, n):
        return jax.random.permutation(self._next(), n)


kernel_name = 'standalone__geglu_ffn__prompt'

def setup_inputs():
    _rng = _Rng(jax.random.key(int.from_bytes(__import__("os").urandom(4), "little")))
    _w = (lambda a: (lambda t: t.astype(jnp.bfloat16) if jnp.issubdtype(t.dtype, jnp.floating) else t)(jnp.asarray(a)))
    B, S, D, F = 1, 2048, 576, 4608
    return {
        "x": _w((lambda *s: _rng.normal(s) * 0.05)(B, S, D)),
        "w_gate": _w((lambda *s: _rng.normal(s) * 0.05)(D, F)),
        "w_up": _w((lambda *s: _rng.normal(s) * 0.05)(D, F)),
        "w_down": _w((lambda *s: _rng.normal(s) * 0.05)(F, D)),
    }

def reference(x, w_gate, w_up, w_down):
    return (_gelu(x @ w_gate) * (x @ w_up)) @ w_down
```

```python
import jax
import jax.numpy as jnp
import numpy as np
import jax.experimental.pallas as pl
import jax.experimental.pallas.tpu as pltpu

_C0 = float(np.sqrt(2.0 / np.pi))
_C1 = 0.044715 * _C0
_NT = (((1,), (1,)), ((), ()))


def _gelu_mul(g, u):
    t = jnp.tanh(g * (_C0 + _C1 * (g * g)))
    return (0.5 * g * u) * (1.0 + t)


@jax.jit
def pallas_standalone__geglu_ffn__prompt_kernel(
    x: jax.Array,
    w_gate: jax.Array,
    w_up: jax.Array,
    w_down: jax.Array,
):
    B, S, D = x.shape
    F = w_gate.shape[1]
    M = B * S
    assert (M, F) == (2048, 4608)
    tm = 512
    cch = (256, 256) + (512,) * 8
    wch = (256, 256, 512, 1024, 2560)
    tjs = (128,) * 4
    nm, nc, nj, nw = M // tm, len(cch), len(tjs), len(wch)
    cb = np.concatenate([[0], np.cumsum(cch)]).tolist()
    wb = np.concatenate([[0], np.cumsum(wch)]).tolist()
    jb = np.concatenate([[0], np.cumsum(tjs)]).tolist()
    G0, U0, D0, X0 = 0, F, 2 * F, 3 * F

    def kern(xT_h, wg_h, wu_h, wdT_h, o_h, buf, x_s, h_s, o_s, sx, sg, su, sd, so):
        def cp(h, lo, n, base, sem):
            return pltpu.make_async_copy(h.at[:, pl.ds(lo, n)], buf.at[:, pl.ds(base + lo, n)], sem)

        cx = lambda m: cp(xT_h, m * tm, tm, X0, sx.at[m])
        cg = lambda i: cp(wg_h, wb[i], wch[i], G0, sg.at[i])
        cu = lambda i: cp(wu_h, wb[i], wch[i], U0, su.at[i])
        cd = cp(wdT_h, 0, F, D0, sd.at[0])

        def co(m, j):
            return pltpu.make_async_copy(
                o_s.at[m, :, pl.ds(jb[j], tjs[j])],
                o_h.at[:, pl.ds(pl.multiple_of(m * tm + jb[j], 128), tjs[j])],
                so.at[m, j])

        cx(0).start()
        for i in range(nw):
            cg(i).start()
            cu(i).start()
        cd.start()
        for m in range(1, nm):
            cx(m).start()

        def tile(m, _):
            first = m == 0
            xx = x_s[m]
            for c in range(nc):
                ws = [i for i in range(nw) if cb[c] <= wb[i] < cb[c + 1]]
                for i in ws:
                    pl.when(first)(cg(i).wait)
                g = jnp.dot(xx, buf[:, pl.ds(G0 + cb[c], cch[c])], preferred_element_type=jnp.float32)
                for i in ws:
                    pl.when(first)(cu(i).wait)
                u = jnp.dot(xx, buf[:, pl.ds(U0 + cb[c], cch[c])], preferred_element_type=jnp.float32)
                h_s[:, pl.ds(cb[c], cch[c])] = _gelu_mul(g, u).astype(h_s.dtype)
            pl.when(first)(cd.wait)
            for j in range(nj):
                o = jax.lax.dot_general(buf[:, pl.ds(D0, F)], h_s[pl.ds(jb[j], tjs[j]), :], _NT,
                                        preferred_element_type=jnp.float32)
                o_s[m, :, pl.ds(jb[j], tjs[j])] = o.astype(o_s.dtype)
                co(m, j).start()
                if j == 0:
                    for mm in range(1, nm):
                        pl.when(first)(cx(mm).wait)
                    mn = jnp.minimum(m + 1, nm - 1)
                    x_s[mn] = buf[:, pl.ds(pl.multiple_of(X0 + mn * tm, 128), tm)].T

        cx(0).wait()
        x_s[0] = buf[:, pl.ds(X0, tm)].T
        jax.lax.fori_loop(0, nm, tile, None)
        for m in range(nm):
            for j in range(nj):
                co(m, j).wait()

    dt = x.dtype
    DMA = pltpu.SemaphoreType.DMA
    oT = pl.pallas_call(
        kern,
        in_specs=[pl.BlockSpec(memory_space=pl.ANY)] * 4,
        out_specs=pl.BlockSpec(memory_space=pl.ANY),
        out_shape=jax.ShapeDtypeStruct((D, M), dt),
        scratch_shapes=[
            pltpu.VMEM((D, 3 * F + M), dt), pltpu.VMEM((nm, tm, D), dt),
            pltpu.VMEM((tm, F), dt), pltpu.VMEM((nm, D, tm), dt),
            DMA((nm,)), DMA((nw,)), DMA((nw,)), DMA((1,)), DMA((nm, nj))],
        compiler_params=pltpu.CompilerParams(
            vmem_limit_bytes=100 * 1024 * 1024,
            flags={"XLA_TPU_RESCHEDULE_DMA_DONES": True}),
    )(x.reshape(M, D).T, w_gate, w_up, w_down.T)
    return oT.T.reshape(B, S, D)
```

```python
import jax
import jax.numpy as jnp
import numpy as np
import jax.experimental.pallas as pl
import jax.experimental.pallas.tpu as pltpu

_C0 = float(np.sqrt(2.0 / np.pi))
_C1 = 0.044715 * _C0
_NT = (((1,), (1,)), ((), ()))

_TM = 512
_TC = 512
_TJ = 128
_XB = 16
_LAST_ROWS = (288, 192, 96)
_W_COPY = (512, 1024)
_PACE_ADDS = 20


def _geglu(g, u):
    t = jnp.tanh(g * (_C0 + _C1 * (g * g)))
    return (g * (0.5 + 0.5 * t)) * u


def _dot(a, b):
    return jnp.dot(a, b, preferred_element_type=jnp.float32)


def _dot_nt(a, b):
    return jax.lax.dot_general(a, b, _NT, preferred_element_type=jnp.float32)


def _offsets(start, sizes):
    return [int(v) for v in start + np.concatenate([[0], np.cumsum(sizes)])]


@jax.jit
def pallas_standalone__geglu_ffn__prompt_kernel(
    x: jax.Array,
    w_gate: jax.Array,
    w_up: jax.Array,
    w_down: jax.Array,
):
    B, S, D = x.shape
    F = w_gate.shape[1]
    M = B * S
    dt = x.dtype
    assert (M, D, F) == (2048, 576, 4608) and dt == jnp.bfloat16
    f32 = jnp.float32
    tm, tc = _TM, _TC
    nm, nj = M // tm, tm // _TJ
    KM = D // 128 * 128
    KR = D - KM
    F1 = F - tc
    k_slices = ((KM, KR), (0, 128), (128, 128), (256, 256))
    nk = len(k_slices)
    w_sizes = _W_COPY + (F1 - tc - sum(_W_COPY),)
    w_lo = _offsets(tc, w_sizes)
    nw = len(w_sizes)
    last_rows = _offsets(0, _LAST_ROWS)
    A0, K0, G0 = 0, 128, 256
    U0, D0, X0 = G0 + F, G0 + 2 * F, G0 + 3 * F
    R0 = X0 + M

    pack = lambda v: pltpu.bitcast(v.astype(dt), jnp.int32)
    unpack = lambda v: pltpu.bitcast(v, dt)

    def kernel(xT_h, wg_h, wu_h, wdT_h, o_h, buf, x_s, h_s, o_s, acc_s, r_s, wr_s,
               o_sem, *xb_s):
        def out_copy(m, j, lo, hi):
            col = pl.multiple_of(m * tm + j * _TJ, 128)
            return pltpu.make_async_copy(
                o_s.at[m, pl.ds(lo, hi - lo), pl.ds(j * _TJ, _TJ)],
                o_h.at[pl.ds(lo, hi - lo), pl.ds(col, _TJ)],
                o_sem.at[0])

        def main(k_sem, g_sem, u_sem, sem):
            def copy(src, r0, nr, c0, nc, dst_col, s):
                return pltpu.make_async_copy(
                    src.at[pl.ds(r0, nr), pl.ds(c0, nc)],
                    buf.at[pl.ds(r0, nr), pl.ds(dst_col, nc)], s)

            xk = [copy(xT_h, r, n, 0, tm, X0, k_sem.at[0, i])
                  for i, (r, n) in enumerate(k_slices)]
            gk = [copy(wg_h, r, n, 0, tc, G0, k_sem.at[1, i])
                  for i, (r, n) in enumerate(k_slices)]
            uk = [copy(wu_h, r, n, 0, tc, U0, k_sem.at[2, i])
                  for i, (r, n) in enumerate(k_slices)]
            gw = [copy(wg_h, 0, D, c, n, G0 + c, g_sem.at[i])
                  for i, (c, n) in enumerate(zip(w_lo, w_sizes))]
            uw = [copy(wu_h, 0, D, c, n, U0 + c, u_sem.at[i])
                  for i, (c, n) in enumerate(zip(w_lo, w_sizes))]
            tails = [copy(wu_h, KM, KR, F1, tc, R0, sem.at[0]),
                     copy(wg_h, KM, KR, F1, tc, R0 + tc, sem.at[1]),
                     copy(xT_h, KM, KR, tm, M - tm, X0 + tm, sem.at[2])]
            x_rest = copy(xT_h, 0, KM, tm, M - tm, X0 + tm, sem.at[3])
            wd_head = copy(wdT_h, 0, D, 0, F1, D0, sem.at[4])
            late = [copy(wg_h, 0, KM, F1, tc, G0 + F1, sem.at[5]),
                    copy(wu_h, 0, KM, F1, tc, U0 + F1, sem.at[6]),
                    copy(wdT_h, 0, D, F1, tc, D0 + F1, sem.at[7])]

            order = [c for i in range(nk) for c in (xk[i], gk[i], uk[i])]
            order += [gw[0], *tails, uw[0]]
            order += [c for i in range(1, nw) for c in (gw[i], uw[i])]
            order += [x_rest, wd_head, *late]
            for c in order:
                c.start()

            def x_slice(m, i):
                r, n = k_slices[i]
                col = X0 + m * tm
                if not isinstance(m, int):
                    col = pl.multiple_of(col, 128)
                return buf[pl.ds(r, n), pl.ds(col, tm)].T

            x_first = buf.at[pl.ds(0, tm), pl.ds(K0, KR)]

            def delay_wait(v, row, i):
                buf[pl.ds(k_slices[i][0] + 16, 16), pl.ds(A0, 128)] = (
                    v[row:row + 16, 0:128].astype(dt))

            def vpu_tail(m):
                never = m < 0
                zero = jnp.minimum(m, 0)
                for q in range(tm // _XB):
                    xr = x_s[pl.ds(q * _XB, _XB), pl.ds(KM, KR)].astype(f32)
                    for k in range(KR):
                        xb_s[q][zero, k % 8, k // 8] = jnp.broadcast_to(
                            xr[:, k:k + 1], (_XB, 128))
                pace = None
                for r in range(0, tm, 8):
                    q, ro = divmod(r, _XB)
                    for n in range(0, 2 * tc, 256):
                        xb = xb_s[q][0, :, :, pl.ds(ro, 8), :].reshape(KR, 8, 128)
                        w = jnp.concatenate([
                            jnp.concatenate([
                                jnp.broadcast_to(
                                    wr_s[:, pl.ds(s, 1), pl.ds(n + c, 128)],
                                    (KR // 8, 8, 128))
                                for s in range(8)], axis=0)
                            for c in (0, 128)], axis=2)
                        acc = jnp.sum(jnp.concatenate([xb, xb], axis=2) * w, axis=0)
                        lo, hi = acc[:, :128], acc[:, 128:]
                        if pace is not None:
                            pace = pltpu.roll(pace, 1, 1)
                            for _ in range(_PACE_ADDS):
                                pace = pace + 1.0
                            lo = jnp.where(never, pace, lo)
                            hi = jnp.where(never, pace, hi)
                        pace = lo + hi
                        r_s[pl.ds(r, 8), pl.ds(n, 256)] = jnp.concatenate([lo, hi], axis=1)

            def row_tile(m, carry):
                def wait(*copies):
                    for c in copies:
                        pl.when(m == 0)(c.wait)

                wait(gk[0])
                xx = x_first[...]
                g = u = None
                for i, (r, n) in enumerate(k_slices):
                    rows = pl.ds(r, n)
                    p = _dot(xx, buf[rows, pl.ds(G0, tc)])
                    g = p if g is None else g + p
                    delay_wait(g, 256, i)
                    wait(uk[i])
                    p = _dot(xx, buf[rows, pl.ds(U0, tc)])
                    u = p if u is None else u + p
                    x_s[:, rows] = xx
                    if i + 1 < nk:
                        delay_wait(u, 128, i + 1)
                        wait(xk[i + 1], gk[i + 1])
                        xx = x_slice(m, i + 1)
                h_s[:, pl.ds(0, tc)] = pack(_geglu(g, u))

                xx = x_s[...]
                for c in range(tc, F1, tc):
                    due = [i for i in range(nw) if w_lo[i] == c]
                    wait(*[gw[i] for i in due])
                    g = _dot(xx, buf[:, pl.ds(G0 + c, tc)])
                    if c == tc:
                        wait(*tails)
                        x_first[...] = x_slice(jnp.minimum(m + 1, nm - 1), 0)
                        wr_s[...] = buf[pl.ds(KM, KR), pl.ds(R0, 2 * tc)].astype(
                            f32).reshape(KR // 8, 8, 2 * tc)
                        vpu_tail(m)
                    wait(*[uw[i] for i in due])
                    u = _dot(xx, buf[:, pl.ds(U0 + c, tc)])
                    h_s[:, pl.ds(c, tc)] = pack(_geglu(g, u))
                    if c == F1 - 3 * tc:
                        wait(x_rest)

                wait(wd_head)
                acc_s[...] = _dot_nt(buf[:, pl.ds(D0, F1)], unpack(h_s[:, pl.ds(0, F1)]))

                wait(*late)
                g = _dot(xx[:, :KM], buf[pl.ds(0, KM), pl.ds(G0 + F1, tc)])
                g = g + r_s[:, pl.ds(tc, tc)]
                u = _dot(xx[:, :KM], buf[pl.ds(0, KM), pl.ds(U0 + F1, tc)])
                u = u + r_s[:, pl.ds(0, tc)]
                h_s[:, pl.ds(F1, tc)] = pack(_geglu(g, u))

                for j in range(nj):
                    cols = pl.ds(j * _TJ, _TJ)
                    h = unpack(h_s[pl.ds(j * _TJ // 2, _TJ // 2), pl.ds(F1, tc)])
                    o = acc_s[:, cols] + _dot_nt(buf[:, pl.ds(D0 + F1, tc)], h)
                    bounds = last_rows if j == nj - 1 else [0, D]
                    for lo, hi in zip(bounds, bounds[1:]):
                        o_s[m, pl.ds(lo, hi - lo), cols] = o[lo:hi].astype(dt)
                        out_copy(m, j, lo, hi).start()
                return carry

            xk[0].wait()
            x_first[...] = x_slice(0, 0)
            jax.lax.fori_loop(0, nm, row_tile, None)

        dma = pltpu.SemaphoreType.DMA
        pl.run_scoped(main, dma((3, nk)), dma((nw,)), dma((nw,)), dma((8,)))
        pltpu.make_async_copy(o_h, o_h, o_sem.at[0]).wait()

    out_t = pl.pallas_call(
        kernel,
        in_specs=[pl.BlockSpec(memory_space=pl.ANY)] * 4,
        out_specs=pl.BlockSpec(memory_space=pl.ANY),
        out_shape=jax.ShapeDtypeStruct((D, M), dt),
        scratch_shapes=[
            pltpu.VMEM((D, R0 + 2 * tc), dt),
            pltpu.VMEM((tm, D), dt),
            pltpu.VMEM((tm // 2, F), jnp.int32),
            pltpu.VMEM((nm, D, tm), dt),
            pltpu.VMEM((D, tm), f32),
            pltpu.VMEM((tm, 2 * tc), f32),
            pltpu.VMEM((KR // 8, 8, 2 * tc), f32),
            pltpu.SemaphoreType.DMA((1,)),
        ] + [pltpu.VMEM((1, 8, KR // 8, _XB, 128), f32)] * (tm // _XB),
        compiler_params=pltpu.CompilerParams(
            vmem_limit_bytes=100 * 1024 * 1024,
            flags={"XLA_TPU_RESCHEDULE_DMA_DONES": True}),
    )(x.reshape(M, D).T, w_gate, w_up, w_down.T)
    return out_t.T.reshape(B, S, D)
```
